```python
import jax
import jax.numpy as jnp

def _softmax(x, axis=-1):
    return jax.nn.softmax(x, axis=axis)

def _gelu(x):
    return jax.nn.gelu(x, approximate=True)

def _silu(x):
    return jax.nn.silu(x)

def _sigmoid(x):
    return jax.nn.sigmoid(x)

def _layernorm(x, axis=-1, eps=1e-05):
    m = jnp.mean(x, axis=axis, keepdims=True)
    v = jnp.var(x, axis=axis, keepdims=True)
    return (x - m) / jnp.sqrt(v + eps)

def _scatter_add(tgt, idx, src, axis=0):
    return tgt.at[idx].add(src)

def _segment_sum(src, seg, n):
    return jax.ops.segment_sum(src, seg, n)

class _Rng:

    def __init__(self, key):
        self._k = key

    def _next(self):
        self._k, sub = jax.random.split(self._k)
        return sub

    def normal(self, shape):
        return jax.random.normal(self._next(), shape, dtype=jnp.bfloat16)

    def randint(self, lo, hi, shape):
        return jax.random.randint(self._next(), shape, lo, hi, dtype=jnp.int32)

    def uniform(self, shape, lo=0.0, hi=1.0):
        return jax.random.uniform(self._next(), shape, jnp.bfloat16, lo, hi)

    def permutation(self, n):
        return jax.random.permutation(self._next(), n)
kernel_name = 'recurrent_scan__ssm_conv_h3__mixer_gmlp__prompt'

def setup_inputs():
    _rng = _Rng(jax.random.key(int.from_bytes(__import__("os").urandom(4), "little")))
    _w = lambda a: (lambda t: t.astype(jnp.bfloat16) if jnp.issubdtype(t.dtype, jnp.floating) else t)(jnp.asarray(a))

    def _A_setup():
        B, S, D = (1, 2048, 640)
        ks = 4
        return {'q': _w((lambda *s: _rng.normal(s) * 0.05)(B, S, D)), 'k': _w((lambda *s: _rng.normal(s) * 0.05)(B, S, D)), 'v': _w((lambda *s: _rng.normal(s) * 0.05)(B, S, D)), 'shift_k': _w((lambda *s: _rng.normal(s) * 0.05)(D, ks) * 0.5), 'ssm_k': _w((lambda *s: _rng.normal(s) * 0.05)(D, S) * (1.0 / S ** 0.5)), 'ssm_D': _w((lambda *s: _rng.normal(s) * 0.05)(D))}
    _A_in = _A_setup()

    def _B_setup():
        B, S, D, F = (1, 2048, 640, 1536)
        Fh = F // 2
        return {'x': _w((lambda *s: _rng.normal(s) * 0.05)(B, S, D)), 'w_in': _w((lambda *s: _rng.normal(s) * 0.05)(D, 2 * Fh)), 'w_sp': _w(0.01 * (lambda *s: _rng.normal(s) * 0.05)(S, S)), 'b_sp': _w(1.0 + 0.01 * (lambda *s: _rng.normal(s) * 0.05)(S)), 'w_out': _w((lambda *s: _rng.normal(s) * 0.05)(Fh, D))}
    _B_in = _B_setup()
    return {'A_q': _A_in['q'], 'A_k': _A_in['k'], 'A_v': _A_in['v'], 'A_shift_k': _A_in['shift_k'], 'A_ssm_k': _A_in['ssm_k'], 'A_ssm_D': _A_in['ssm_D'], 'B_x': _B_in['x'], 'B_w_in': _B_in['w_in'], 'B_w_sp': _B_in['w_sp'], 'B_b_sp': _B_in['b_sp'], 'B_w_out': _B_in['w_out']}

def reference(A_q, A_k, A_v, A_shift_k, A_ssm_k, A_ssm_D, B_x, B_w_in, B_w_sp, B_b_sp, B_w_out):

    def _A_ref(q, k, v, shift_k, ssm_k, ssm_D):
        B, S, D = q.shape
        ks = shift_k.shape[-1]
        k_pad = jnp.pad(k, ((0, 0), (ks - 1, 0), (0, 0)))
        k_shift = jnp.zeros_like(k)
        for t in range(ks):
            k_shift = k_shift + k_pad[:, t:t + S, :] * shift_k[:, ks - 1 - t][None, None, :]
        kv = k_shift * v
        L = 2 * S
        kv_pad = jnp.pad(kv, ((0, 0), (0, S), (0, 0)))
        kf_pad = jnp.pad(ssm_k, ((0, 0), (0, S)))
        kv_f = (lambda x, axes=(-2, -1): jnp.fft.rfft2(x.astype(jnp.float32), axes=axes))(kv_pad[:, None, :, :], axes=(1, 2))
        kf_f = (lambda x, axes=(-2, -1): jnp.fft.rfft2(x.astype(jnp.float32), axes=axes))(kf_pad[:, None, :], axes=(1, 2))
        kf_f = (lambda x, *d: x.transpose(*d))(kf_f, 1, 2, 0)
        y_f = kv_f * kf_f[None, :, :, :]
        y = (lambda x, s, axes=(-2, -1): jnp.fft.irfft2(x, s=s, axes=axes).astype(jnp.bfloat16))(y_f, (1, L), axes=(1, 2))[:, 0, :S, :]
        y = y + kv * ssm_D[None, None, :]
        return q * y

    def _B_ref(x, w_in, w_sp, b_sp, w_out):
        B, S, D = x.shape
        F = w_in.shape[-1]
        Fh = F // 2
        z = _gelu(jnp.einsum('bsd,df->bsf', x, w_in))
        z1 = z[..., :Fh].copy()
        z2 = _layernorm(z[..., Fh:], axis=-1)
        g = jnp.einsum('ts,bsf->btf', w_sp, z2) + b_sp[None, :, None]
        return jnp.einsum('bsf,fd->bsd', z1 * g, w_out)
    x = A_q
    xn = _layernorm(x, axis=-1)
    s = _A_ref(xn, A_k, A_v, A_shift_k, A_ssm_k, A_ssm_D)
    g = _silu(_B_ref(xn, B_w_in, B_w_sp, B_b_sp, B_w_out))
    return x + s * g
```

```python
import math

import jax
import jax.numpy as jnp
import numpy as np
from jax import lax
import jax.experimental.pallas as pl
import jax.experimental.pallas.tpu as pltpu

S, D, FH = 2048, 640, 768
N1, N2 = 32, 128
NB = N1 // 2
NS = 8
RB = S // NS
RR = N2 // NS
DR = D // NS
NC = D // 128
F32, BF16 = jnp.float32, jnp.bfloat16


def _dft_mats():
    k1 = np.arange(NB + 1)[:, None, None]
    k2 = np.arange(N2)[None, :, None]
    n2 = np.arange(N2)[None, None, :]
    m = np.exp(-2j * np.pi * (n2 * k1 / (N1 * N2) + n2 * k2 / N2))
    f = np.concatenate([np.concatenate([m.real, -m.imag], 2),
                        np.concatenate([m.imag, m.real], 2)], 1)
    g = np.transpose(f, (0, 2, 1)) / (N1 * N2)
    return f.astype(np.float32), g.astype(np.float32)


_F, _G = _dft_mats()


def _add(a, b):
    return b if a is None else a if b is None else a + b


def _sub(a, b):
    return (None if b is None else -b) if a is None else a if b is None else a - b


def _cmul(re, im, ang):
    c, s = float(np.float32(math.cos(ang))), float(np.float32(math.sin(ang)))
    if im is None:
        return re * c, re * s
    if abs(abs(c) - abs(s)) < 1e-6:
        if c * s > 0:
            return (re - im) * c, (re + im) * c
        return (re + im) * c, (im - re) * c
    return re * c - im * s, re * s + im * c


def _rfft(x):
    n = len(x)
    if n == 2:
        return [(_add(x[0], x[1]), None), (_sub(x[0], x[1]), None)]
    e, o = _rfft(x[0::2]), _rfft(x[1::2])
    h = n // 2
    out = [None] * (h + 1)
    out[0] = (e[0][0] + o[0][0], None)
    out[h] = (e[0][0] - o[0][0], None)
    q = h // 2
    out[q] = (e[q][0], -o[q][0])
    for k in range(1, q):
        tr, ti = _cmul(o[k][0], o[k][1], -2 * math.pi * k / n)
        er, ei = e[k]
        out[k] = (er + tr, ei + ti)
        out[h - k] = (er - tr, ti - ei)
    return out


def _irfft_half(X):
    n = 2 * (len(X) - 1)
    if n == 2:
        return [X[0][0] + X[1][0]]
    h, q = n // 2, n // 4
    e, o = [None] * (q + 1), [None] * (q + 1)
    e[0] = (X[0][0] + X[h][0], None)
    o[0] = (X[0][0] - X[h][0], None)
    e[q] = (X[q][0] * 2.0, None)
    o[q] = (X[q][1] * -2.0, None)
    for k in range(1, q):
        (ar, ai), (br, bi) = X[k], X[h - k]
        e[k] = (ar + br, ai - bi)
        o[k] = _cmul(ar - br, ai + bi, 2 * math.pi * k / n)
    xe, xo = _irfft_half(e), _irfft_half(o)
    out = [None] * h
    out[0::2], out[1::2] = xe, xo
    return out[:h]


def _irfft_first(X):
    n = 2 * (len(X) - 1)
    full = _irfft_full(X)
    return full[: n // 2]


def _irfft_full(X, need=None):
    n = 2 * (len(X) - 1)
    need = n // 2 if need is None else need
    if n == 2:
        r = [X[0][0] + X[1][0]]
        if need > 1:
            r.append(X[0][0] - X[1][0])
        return r
    h, q = n // 2, n // 4
    e, o = [None] * (q + 1), [None] * (q + 1)
    e[0] = (X[0][0] + X[h][0], None)
    o[0] = (X[0][0] - X[h][0], None)
    e[q] = (X[q][0] * 2.0, None)
    o[q] = (X[q][1] * -2.0, None)
    for k in range(1, q):
        (ar, ai), (br, bi) = X[k], X[h - k]
        e[k] = (ar + br, ai - bi)
        o[k] = _cmul(ar - br, ai + bi, 2 * math.pi * k / n)
    xe, xo = _irfft_full(e, need // 2), _irfft_full(o, need // 2)
    out = [None] * need
    out[0::2], out[1::2] = xe, xo
    return out


def _ln(x):
    m = jnp.mean(x, axis=-1, keepdims=True)
    c = x - m
    v = jnp.mean(c * c, axis=-1, keepdims=True)
    return c * lax.rsqrt(v + 1e-5)


def _gelu(x):
    return 0.5 * x * (1.0 + jnp.tanh(0.7978845608028654 * (x + 0.044715 * x * x * x)))


def _dot(a, b):
    return jnp.dot(a, b, preferred_element_type=F32)


def _dot_nt(a, b):
    return lax.dot_general(a, b, (((1,), (1,)), ((), ())), preferred_element_type=F32)


def _freq_unit(f, g, ak, af):
    xk = _dot(f, ak)
    xf = _dot_nt(f, af)
    kr, ki, fr, fi = xk[:N2], xk[N2:], xf[:N2], xf[N2:]
    y = jnp.concatenate([kr * fr - ki * fi, kr * fi + ki * fr], 0).astype(BF16)
    return _dot(g, y)


def _kernel(q1_ref, k_ref, kh_ref, v_ref, sk_ref, shift_ref, ssmd_ref, win_ref,
            wsp_ref, bsp_ref, f_ref, g_ref, f0_ref, g0_ref, q3_ref, wout_ref,
            o_ref,
            z1_s, z2_s, ak_s, af_s, zz_s, kv_s):
    step = pl.program_id(0)

    @pl.when(step < NS)
    def _phase1():
        r = step
        row0 = pl.multiple_of(r * RB, RB)
        xn = _ln(q1_ref[...].astype(F32)).astype(BF16)
        z = _gelu(_dot(xn, win_ref[...]))
        z1_s[pl.ds(row0, RB), :] = z[:, :FH].astype(BF16)
        z2_s[pl.ds(row0, RB), :] = _ln(z[:, FH:]).astype(BF16)

        rr = pl.multiple_of(r * RR, RR)
        first = r == 0
        for c in range(NC):
            ls = slice(c * 128, (c + 1) * 128)
            w = shift_ref[:, ls].astype(F32)
            kvs = []
            for n1 in range(NB):
                cur = k_ref[n1, :, ls].astype(F32)
                prev = kh_ref[n1, 8:, ls].astype(F32)
                if n1 == 0:
                    prev = jnp.where(first, 0.0, prev)
                else:
                    prev = jnp.where(first, kh_ref[n1 - 1, 8:, ls].astype(F32), prev)
                ext = jnp.concatenate([prev, cur], 0)
                ks = cur * w[0:1]
                for j in range(1, 4):
                    ks = ks + ext[8 - j:8 - j + RR] * w[j:j + 1]
                kv = ks * v_ref[n1, :, ls].astype(F32)
                kvs.append(kv)
                kv_s[n1, pl.ds(rr, RR), ls] = kv.astype(BF16)
            X = _rfft(kvs + [None] * NB)
            for k1 in range(NB + 1):
                re, im = X[k1]
                ak_s[k1, pl.ds(rr, RR), ls] = re.astype(BF16)
                im = jnp.zeros_like(re) if im is None else im
                ak_s[k1, pl.ds(N2 + rr, RR), ls] = im.astype(BF16)
        for c in range(DR // 16):
            d0 = pl.multiple_of(r * DR + c * 16, 16)
            xs = [sk_ref[c * 16:(c + 1) * 16, n1 * N2:(n1 + 1) * N2].astype(F32) for n1 in range(NB)]
            X = _rfft(xs + [None] * NB)
            for k1 in range(NB + 1):
                re, im = X[k1]
                af_s[k1, pl.ds(d0, 16), :N2] = re.astype(BF16)
                im = jnp.zeros_like(re) if im is None else im
                af_s[k1, pl.ds(d0, 16), N2:] = im.astype(BF16)

    @pl.when(step == NS)
    def _unit0():
        zz_s[0] = _freq_unit(f0_ref[0], g0_ref[0], ak_s[0], af_s[0])

    @pl.when(jnp.logical_and(step >= NS, step < 2 * NS))
    def _phase2():
        r = step - NS
        row0 = pl.multiple_of(r * RB, RB)
        gate = _dot(wsp_ref[...], z2_s[...]) + bsp_ref[...].astype(F32)
        z1_s[pl.ds(row0, RB), :] = (z1_s[pl.ds(row0, RB), :].astype(F32) * gate).astype(BF16)
        for u in range(2):
            k1 = 2 * r + u + 1
            zz_s[k1] = _freq_unit(f_ref[u], g_ref[u], ak_s[k1], af_s[k1])

    @pl.when(step >= 2 * NS)
    def _phase3():
        r = step - 2 * NS
        rr = pl.multiple_of(r * RR, RR)
        h = jnp.concatenate([z1_s[pl.ds(n1 * N2 + rr, RR), :] for n1 in range(NB)], 0)
        o = _dot(h, wout_ref[...])
        gate = o * jax.nn.sigmoid(o)
        x = q3_ref[...].reshape(NB * RR, D).astype(F32)
        xg = _ln(x) * gate
        for c in range(NC):
            ls = slice(c * 128, (c + 1) * 128)
            X = [(zz_s[k1, pl.ds(rr, RR), ls], zz_s[k1, pl.ds(N2 + rr, RR), ls]) for k1 in range(NB + 1)]
            ys = _irfft_full(X)
            dd = ssmd_ref[:, ls].astype(F32)
            for n1 in range(NB):
                y = ys[n1] + kv_s[n1, pl.ds(rr, RR), ls].astype(F32) * dd
                rs = slice(n1 * RR, (n1 + 1) * RR)
                o_ref[n1, :, ls] = (x[rs, ls] + y * xg[rs, ls]).astype(o_ref.dtype)


@jax.jit
def pallas_recurrent_scan__ssm_conv_h3__mixer_gmlp__prompt_kernel(
    A_q: jax.Array,
    A_k: jax.Array,
    A_v: jax.Array,
    A_shift_k: jax.Array,
    A_ssm_k: jax.Array,
    A_ssm_D: jax.Array,
    B_x: jax.Array,
    B_w_in: jax.Array,
    B_w_sp: jax.Array,
    B_b_sp: jax.Array,
    B_w_out: jax.Array,
):
    del B_x
    q2 = A_q.reshape(S, D)
    tiled = lambda a: a.reshape(NB, NS, RR, D)
    f = jnp.asarray(_F, BF16)
    g = jnp.asarray(_G, BF16)

    p1 = lambda i: jnp.minimum(i, NS - 1)
    p2 = lambda i: jnp.clip(i - NS, 0, NS - 1)
    p3 = lambda i: jnp.clip(i - 2 * NS, 0, NS - 1)
    tspec = lambda m: pl.BlockSpec((NB, None, RR, D), lambda i: (0, m(i), 0, 0))
    const = lambda shape: pl.BlockSpec(shape, lambda i: (0,) * len(shape))

    out = pl.pallas_call(
        _kernel,
        grid=(3 * NS,),
        in_specs=[
            pl.BlockSpec((RB, D), lambda i: (p1(i), 0)),
            tspec(p1),
            tspec(lambda i: (p1(i) + NS - 1) % NS),
            tspec(p1),
            pl.BlockSpec((DR, S), lambda i: (p1(i), 0)),
            const((4, D)),
            const((1, D)),
            const((D, 2 * FH)),
            pl.BlockSpec((RB, S), lambda i: (p2(i), 0)),
            pl.BlockSpec((RB, 1), lambda i: (p2(i), 0)),
            pl.BlockSpec((2, 2 * N2, 2 * N2), lambda i: (p2(i), 0, 0)),
            pl.BlockSpec((2, 2 * N2, 2 * N2), lambda i: (p2(i), 0, 0)),
            const((1, 2 * N2, 2 * N2)),
            const((1, 2 * N2, 2 * N2)),
            tspec(p3),
            const((FH, D)),
        ],
        out_specs=tspec(p3),
        out_shape=jax.ShapeDtypeStruct((NB, NS, RR, D), A_q.dtype),
        scratch_shapes=[
            pltpu.VMEM((S, FH), BF16),
            pltpu.VMEM((S, FH), BF16),
            pltpu.VMEM((NB + 1, 2 * N2, D), BF16),
            pltpu.VMEM((NB + 1, D, 2 * N2), BF16),
            pltpu.VMEM((NB + 1, 2 * N2, D), F32),
            pltpu.VMEM((NB, N2, D), BF16),
        ],
        compiler_params=pltpu.CompilerParams(
            dimension_semantics=("arbitrary",),
            vmem_limit_bytes=110 * 1024 * 1024,
        ),
    )(q2, tiled(A_k), tiled(A_k), tiled(A_v), A_ssm_k, A_shift_k.T, A_ssm_D.reshape(1, D),
      B_w_in, B_w_sp, B_b_sp.reshape(S, 1), f[1:], g[1:], f[:1], g[:1], tiled(A_q), B_w_out)
    return out.reshape(A_q.shape)
```

```python
import math

import jax
import jax.numpy as jnp
import numpy as np
from jax import lax
import jax.experimental.pallas as pl
import jax.experimental.pallas.tpu as pltpu

S, D, FH = 2048, 640, 768
N1, N2 = 64, 64
NB = N1 // 2
NK = NB + 1
NC = D // 128
P1, P2, P3 = 8, 16, 8
RB = S // P1
RS = S // P2
F32, BF16 = jnp.float32, jnp.bfloat16


def _dft_mats():
    k1 = np.arange(NK)[:, None, None]
    k2 = np.arange(N2)[None, :, None]
    n2 = np.arange(N2)[None, None, :]
    m = np.exp(-2j * np.pi * (n2 * k1 / (N1 * N2) + n2 * k2 / N2))
    f = np.concatenate([np.concatenate([m.real, -m.imag], 2),
                        np.concatenate([m.imag, m.real], 2)], 1)
    perm = np.array([part * N2 + 8 * g + i for g in range(N2 // 8) for part in range(2) for i in range(8)])
    f = f[:, :, perm]
    g = np.transpose(f, (0, 2, 1)) / (N1 * N2)
    return f.astype(np.float32), g.astype(np.float32)


_F, _G = _dft_mats()


def _add(a, b):
    return b if a is None else a if b is None else a + b


def _sub(a, b):
    return (None if b is None else -b) if a is None else a if b is None else a - b


def _cmul(re, im, ang):
    c, s = float(np.float32(math.cos(ang))), float(np.float32(math.sin(ang)))
    if im is None:
        return re * c, re * s
    if abs(abs(c) - abs(s)) < 1e-6:
        if c * s > 0:
            return (re - im) * c, (re + im) * c
        return (re + im) * c, (im - re) * c
    return re * c - im * s, re * s + im * c


def _rfft(x):
    n = len(x)
    if n == 2:
        return [(_add(x[0], x[1]), None), (_sub(x[0], x[1]), None)]
    e, o = _rfft(x[0::2]), _rfft(x[1::2])
    h = n // 2
    out = [None] * (h + 1)
    out[0] = (e[0][0] + o[0][0], None)
    out[h] = (e[0][0] - o[0][0], None)
    q = h // 2
    out[q] = (e[q][0], -o[q][0])
    for k in range(1, q):
        tr, ti = _cmul(o[k][0], o[k][1], -2 * math.pi * k / n)
        er, ei = e[k]
        out[k] = (er + tr, ei + ti)
        out[h - k] = (er - tr, ti - ei)
    return out


def _irfft_full(X, need=None):
    n = 2 * (len(X) - 1)
    need = n // 2 if need is None else need
    if n == 2:
        r = [X[0][0] + X[1][0]]
        if need > 1:
            r.append(X[0][0] - X[1][0])
        return r
    h, q = n // 2, n // 4
    e, o = [None] * (q + 1), [None] * (q + 1)
    e[0] = (X[0][0] + X[h][0], None)
    o[0] = (X[0][0] - X[h][0], None)
    e[q] = (X[q][0] * 2.0, None)
    o[q] = (X[q][1] * -2.0, None)
    for k in range(1, q):
        (ar, ai), (br, bi) = X[k], X[h - k]
        e[k] = (ar + br, ai - bi)
        o[k] = _cmul(ar - br, ai + bi, 2 * math.pi * k / n)
    xe, xo = _irfft_full(e, need // 2), _irfft_full(o, need // 2)
    out = [None] * need
    out[0::2], out[1::2] = xe, xo
    return out


def _ln(x):
    m = jnp.mean(x, axis=-1, keepdims=True)
    c = x - m
    v = jnp.mean(c * c, axis=-1, keepdims=True)
    return c * lax.rsqrt(v + 1e-5)


def _gelu(x):
    return 0.5 * x * (1.0 + jnp.tanh(0.7978845608028654 * (x + 0.044715 * x * x * x)))


def _dot(a, b):
    return jnp.dot(a, b, preferred_element_type=F32)


def _kernel(q_ref, k_ref, v_ref, sk_ref, shift_ref, ssmd_ref, win_ref, wsp_ref, bsp_ref,
            f_hbm, g_hbm, wout_hbm,
            o_ref,
            z1_s, z2_s, xn_s, x_s, a_s, zz_s, s_s, tail_s, f_s, g_s, wout_s, sem):
    step = pl.program_id(0)
    copies = [pltpu.make_async_copy(f_hbm, f_s, sem.at[0]),
              pltpu.make_async_copy(g_hbm, g_s, sem.at[1]),
              pltpu.make_async_copy(wout_hbm, wout_s, sem.at[2])]

    @pl.when(step == 0)
    def _start():
        for cp in copies:
            cp.start()
        tail_s[...] = jnp.zeros_like(tail_s)

    @pl.when(step < P1)
    def _phase1():
        row0 = pl.multiple_of(step * RB, RB)
        rows = pl.ds(row0, RB)
        xn = _ln(q_ref[...].astype(F32)).astype(BF16)
        xn_s[rows, :] = xn
        z = _gelu(_dot(xn, win_ref[...]))
        z1_s[rows, :] = z[:, :FH].astype(BF16)
        z2_s[rows, :] = _ln(z[:, FH:]).astype(BF16)
        kf = k_ref[...].astype(F32)
        w = shift_ref[...].astype(F32)
        ext = jnp.concatenate([tail_s[...], kf], 0)
        ks = kf * w[0:1]
        for j in range(1, 4):
            ks = ks + ext[8 - j:8 - j + RB] * w[j:j + 1]
        tail_s[...] = kf[RB - 8:]
        x_s[0, rows, :] = ks * v_ref[...].astype(F32)
        x_s[1, rows, :] = sk_ref[...].astype(F32).T

    def spatial():
        r = step - P1
        rows = pl.ds(pl.multiple_of(r * RS, RS), RS)
        b = bsp_ref[...].astype(F32)
        bcol = jnp.broadcast_to(b, (RS, RS)).T
        gate = _dot(wsp_ref[...], z2_s[...]) + jnp.concatenate([bcol] * (FH // RS), 1)
        z1_s[rows, :] = (z1_s[rows, :].astype(F32) * gate).astype(BF16)

    @pl.when(jnp.logical_and(step >= P1, step < P1 + 8))
    def _phase2a():
        spatial()
        r = step - P1
        which = r // 4
        for gg in range(2):
            g8 = (r % 4) * 2 + gg
            for c in range(NC):
                ls = slice(c * 128, (c + 1) * 128)
                xs = [x_s[which, pl.ds(pl.multiple_of(n1 * N2 + g8 * 8, 8), 8), ls] for n1 in range(NB)]
                X = _rfft(xs + [None] * NB)
                for k1 in range(NK):
                    re, im = X[k1]
                    im = jnp.zeros_like(re) if im is None else im
                    a_s[which, k1, pl.ds(pl.multiple_of(g8 * 16, 16), 16), ls] = (
                        jnp.concatenate([re, im], 0).astype(BF16))

    @pl.when(step == P1 + 8)
    def _wait_fg():
        copies[0].wait()
        copies[1].wait()

    @pl.when(jnp.logical_and(step >= P1 + 8, step < P1 + 11))
    def _phase2b():
        spatial()
        r = step - (P1 + 8)
        for u in range(11):
            k1 = r * 11 + u
            f = f_s[k1]
            xk = _dot(f, a_s[0, k1])
            xf = _dot(f, a_s[1, k1])
            kr, ki, fr, fi = xk[:N2], xk[N2:], xf[:N2], xf[N2:]
            y = jnp.concatenate([kr * fr - ki * fi, kr * fi + ki * fr], 0).astype(BF16)
            zz_s[k1] = _dot(g_s[k1], y)

    @pl.when(jnp.logical_and(step >= P1 + 11, step < P1 + 15))
    def _phase2c():
        spatial()
        r = step - (P1 + 11)
        for gg in range(2):
            g8 = r * 2 + gg
            for c in range(NC):
                ls = slice(c * 128, (c + 1) * 128)
                X = [(zz_s[k1, pl.ds(pl.multiple_of(g8 * 16, 16), 8), ls],
                      zz_s[k1, pl.ds(pl.multiple_of(g8 * 16 + 8, 8), 8), ls]) for k1 in range(NK)]
                ys = _irfft_full(X)
                dd = ssmd_ref[:, ls].astype(F32)
                for n1 in range(NB):
                    rows = pl.ds(pl.multiple_of(n1 * N2 + g8 * 8, 8), 8)
                    s_s[rows, ls] = ys[n1] + x_s[0, rows, ls] * dd

    @pl.when(step == P1 + 15)
    def _phase2d():
        spatial()
        copies[2].wait()

    @pl.when(step >= P1 + P2)
    def _phase3():
        rows = pl.ds(pl.multiple_of((step - P1 - P2) * RB, RB), RB)
        o = _dot(z1_s[rows, :], wout_s[...])
        gate = o * jax.nn.sigmoid(o)
        o_ref[...] = (q_ref[...].astype(F32)
                      + xn_s[rows, :].astype(F32) * s_s[rows, :] * gate).astype(o_ref.dtype)


@jax.jit
def pallas_recurrent_scan__ssm_conv_h3__mixer_gmlp__prompt_kernel(
    A_q: jax.Array,
    A_k: jax.Array,
    A_v: jax.Array,
    A_shift_k: jax.Array,
    A_ssm_k: jax.Array,
    A_ssm_D: jax.Array,
    B_x: jax.Array,
    B_w_in: jax.Array,
    B_w_sp: jax.Array,
    B_b_sp: jax.Array,
    B_w_out: jax.Array,
):
    del B_x
    f = jnp.asarray(_F, BF16)
    g = jnp.asarray(_G, BF16)

    p1 = lambda i: jnp.minimum(i, P1 - 1)
    p2 = lambda i: jnp.clip(i - P1, 0, P2 - 1)
    p3 = lambda i: jnp.clip(i - P1 - P2, 0, P3 - 1)
    p13 = lambda i: jnp.where(i < P1 + P2, p1(i), p3(i))
    const = lambda shape: pl.BlockSpec(shape, lambda i: (0,) * len(shape))
    hbm = pl.BlockSpec(memory_space=pl.ANY)

    out = pl.pallas_call(
        _kernel,
        grid=(P1 + P2 + P3,),
        in_specs=[
            pl.BlockSpec((RB, D), lambda i: (p13(i), 0)),
            pl.BlockSpec((RB, D), lambda i: (p1(i), 0)),
            pl.BlockSpec((RB, D), lambda i: (p1(i), 0)),
            pl.BlockSpec((D, RB), lambda i: (0, p1(i))),
            const((4, D)),
            const((1, D)),
            const((D, 2 * FH)),
            pl.BlockSpec((RS, S), lambda i: (p2(i), 0)),
            pl.BlockSpec((None, 1, RS), lambda i: (p2(i), 0, 0)),
            hbm, hbm, hbm,
        ],
        out_specs=pl.BlockSpec((RB, D), lambda i: (p3(i), 0)),
        out_shape=jax.ShapeDtypeStruct((S, D), A_q.dtype),
        scratch_shapes=[
            pltpu.VMEM((S, FH), BF16),
            pltpu.VMEM((S, FH), BF16),
            pltpu.VMEM((S, D), BF16),
            pltpu.VMEM((2, S, D), F32),
            pltpu.VMEM((2, NK, 2 * N2, D), BF16),
            pltpu.VMEM((NK, 2 * N2, D), F32),
            pltpu.VMEM((S, D), F32),
            pltpu.VMEM((8, D), F32),
            pltpu.VMEM((NK, 2 * N2, 2 * N2), BF16),
            pltpu.VMEM((NK, 2 * N2, 2 * N2), BF16),
            pltpu.VMEM((FH, D), BF16),
            pltpu.SemaphoreType.DMA((3,)),
        ],
        compiler_params=pltpu.CompilerParams(
            dimension_semantics=("arbitrary",),
            vmem_limit_bytes=110 * 1024 * 1024,
        ),
    )(A_q.reshape(S, D), A_k.reshape(S, D), A_v.reshape(S, D), A_ssm_k, A_shift_k.T,
      A_ssm_D.reshape(1, D), B_w_in, B_w_sp, B_b_sp.reshape(P2, 1, RS), f, g, B_w_out)
    return out.reshape(A_q.shape)
```

```python
import functools
import math

import jax
import jax.numpy as jnp
import numpy as np
from jax import lax
import jax.experimental.pallas as pl
import jax.experimental.pallas.tpu as pltpu

S, D, FH = 2048, 640, 768
N1, N2 = 64, 64
NB = N1 // 2
NK = NB + 1
NC = D // 128
P1, P2, P3 = 8, 16, 8
RB = S // P1
RS = S // P2
F32, BF16 = jnp.float32, jnp.bfloat16


def _dft_mats():
    k1 = np.arange(NK)[:, None, None]
    k2 = np.arange(N2)[None, :, None]
    n2 = np.arange(N2)[None, None, :]
    m = np.exp(-2j * np.pi * (n2 * k1 / (N1 * N2) + n2 * k2 / N2))
    f = np.concatenate([np.concatenate([m.real, -m.imag], 2),
                        np.concatenate([m.imag, m.real], 2)], 1)
    perm = np.array([part * N2 + 8 * g + i for g in range(N2 // 8) for part in range(2) for i in range(8)])
    f = f[:, :, perm]
    g = np.transpose(f, (0, 2, 1)) / (N1 * N2)
    return f.astype(np.float32), g.astype(np.float32)


_F, _G = _dft_mats()


def _add(a, b):
    return b if a is None else a if b is None else a + b


def _sub(a, b):
    return (None if b is None else -b) if a is None else a if b is None else a - b


def _cmul(re, im, ang):
    c, s = float(np.float32(math.cos(ang))), float(np.float32(math.sin(ang)))
    if im is None:
        return re * c, re * s
    if abs(abs(c) - abs(s)) < 1e-6:
        if c * s > 0:
            return (re - im) * c, (re + im) * c
        return (re + im) * c, (im - re) * c
    return re * c - im * s, re * s + im * c


def _rfft(x):
    n = len(x)
    if n == 2:
        return [(_add(x[0], x[1]), None), (_sub(x[0], x[1]), None)]
    e, o = _rfft(x[0::2]), _rfft(x[1::2])
    h = n // 2
    out = [None] * (h + 1)
    out[0] = (e[0][0] + o[0][0], None)
    out[h] = (e[0][0] - o[0][0], None)
    q = h // 2
    out[q] = (e[q][0], -o[q][0])
    for k in range(1, q):
        tr, ti = _cmul(o[k][0], o[k][1], -2 * math.pi * k / n)
        er, ei = e[k]
        out[k] = (er + tr, ei + ti)
        out[h - k] = (er - tr, ti - ei)
    return out


def _irfft_full(X, need=None):
    n = 2 * (len(X) - 1)
    need = n // 2 if need is None else need
    if n == 2:
        r = [X[0][0] + X[1][0]]
        if need > 1:
            r.append(X[0][0] - X[1][0])
        return r
    h, q = n // 2, n // 4
    e, o = [None] * (q + 1), [None] * (q + 1)
    e[0] = (X[0][0] + X[h][0], None)
    o[0] = (X[0][0] - X[h][0], None)
    e[q] = (X[q][0] * 2.0, None)
    o[q] = (X[q][1] * -2.0, None)
    for k in range(1, q):
        (ar, ai), (br, bi) = X[k], X[h - k]
        e[k] = (ar + br, ai - bi)
        o[k] = _cmul(ar - br, ai + bi, 2 * math.pi * k / n)
    xe, xo = _irfft_full(e, need // 2), _irfft_full(o, need // 2)
    out = [None] * need
    out[0::2], out[1::2] = xe, xo
    return out


def _ln(x):
    m = jnp.mean(x, axis=-1, keepdims=True)
    c = x - m
    v = jnp.mean(c * c, axis=-1, keepdims=True)
    return c * lax.rsqrt(v + 1e-5)


def _gelu(x):
    return 0.5 * x * (1.0 + jnp.tanh(0.7978845608028654 * (x + 0.044715 * x * x * x)))


def _dot(a, b):
    return jnp.dot(a, b, preferred_element_type=F32)


def _kernel(q_ref, k_ref, v_ref, sk_ref, shift_ref, ssmd_ref, win_ref, wsp_ref, bsp_ref,
            f_hbm, g_hbm, wout_hbm,
            o_ref,
            z1_s, z2_s, xn_s, x_s, a_s, zz_s, s_s, tail_s, f_s, g_s, wout_s, sem):
    step = pl.program_id(0)
    copies = [pltpu.make_async_copy(f_hbm, f_s, sem.at[0]),
              pltpu.make_async_copy(g_hbm, g_s, sem.at[1]),
              pltpu.make_async_copy(wout_hbm, wout_s, sem.at[2])]

    @pl.when(step == 0)
    def _start():
        tail_s[...] = jnp.zeros_like(tail_s)

    @pl.when(step == 1)
    def _start2():
        for cp in copies:
            cp.start()

    @pl.when(step < P1)
    def _phase1():
        row0 = pl.multiple_of(step * RB, RB)
        rows = pl.ds(row0, RB)
        w = shift_ref[...].astype(F32)

        def gmlp(h):
            hr = pl.ds(pl.multiple_of(step * RB + h * 128, 128), 128)
            xn = _ln(q_ref[h * 128:(h + 1) * 128, :].astype(F32)).astype(BF16)
            xn_s[hr, :] = xn
            z1_s[hr, :] = _gelu(_dot(xn, win_ref[:, :FH])).astype(BF16)
            return lambda: z2_s.__setitem__((hr, slice(None)),
                                            _ln(_gelu(_dot(xn, win_ref[:, FH:]))).astype(BF16))

        def kv(h):
            hr = pl.ds(pl.multiple_of(step * RB + h * 128, 128), 128)
            kf = k_ref[h * 128:(h + 1) * 128, :].astype(F32)
            ext = jnp.concatenate([tail_s[...], kf], 0)
            ks = kf * w[0:1]
            for j in range(1, 4):
                ks = ks + ext[8 - j:8 - j + 128] * w[j:j + 1]
            tail_s[...] = kf[120:]
            x_s[0, hr, :] = ks * v_ref[h * 128:(h + 1) * 128, :].astype(F32)
            x_s[1, hr, :] = sk_ref[:, h * 128:(h + 1) * 128].astype(F32).T

        for h in range(2):
            rest = gmlp(h)
            kv(h)
            rest()

    def spatial_parts(n):
        r = step - P1
        rows = pl.ds(pl.multiple_of(r * RS, RS), RS)
        bcol = jnp.broadcast_to(bsp_ref[...].astype(F32), (RS, RS)).T
        wd = FH // n

        def part(j):
            cs = slice(j * wd, (j + 1) * wd)
            gate = _dot(wsp_ref[...], z2_s[:, cs]) + jnp.concatenate([bcol] * (wd // RS), 1)
            z1_s[rows, cs] = (z1_s[rows, cs].astype(F32) * gate).astype(BF16)
        return [functools.partial(part, j) for j in range(n)]

    def spatial():
        spatial_parts(1)[0]()

    @pl.when(jnp.logical_and(step >= P1, step < P1 + 8))
    def _phase2a():
        parts = spatial_parts(6)
        r = step - P1
        which = r // 4
        for gg in range(2):
            g8 = (r % 4) * 2 + gg
            for c in range(NC):
                if parts and (gg * NC + c) in (0, 1, 3, 5, 6, 8):
                    parts.pop(0)()
                ls = slice(c * 128, (c + 1) * 128)
                xs = [x_s[which, pl.ds(pl.multiple_of(n1 * N2 + g8 * 8, 8), 8), ls] for n1 in range(NB)]
                X = _rfft(xs + [None] * NB)
                for k1 in range(NK):
                    re, im = X[k1]
                    im = jnp.zeros_like(re) if im is None else im
                    a_s[which, k1, pl.ds(pl.multiple_of(g8 * 16, 16), 16), ls] = (
                        jnp.concatenate([re, im], 0).astype(BF16))

    @pl.when(step == P1 + 8)
    def _wait_fg():
        copies[0].wait()
        copies[1].wait()

    @pl.when(jnp.logical_and(step >= P1 + 8, step < P1 + 11))
    def _phase2b():
        spatial()
        r = step - (P1 + 8)
        for u in range(11):
            k1 = r * 11 + u
            f = f_s[k1]
            xk = _dot(f, a_s[0, k1])
            xf = _dot(f, a_s[1, k1])
            kr, ki, fr, fi = xk[:N2], xk[N2:], xf[:N2], xf[N2:]
            y = jnp.concatenate([kr * fr - ki * fi, kr * fi + ki * fr], 0).astype(BF16)
            zz_s[k1] = _dot(g_s[k1], y)

    @pl.when(jnp.logical_and(step >= P1 + 11, step < P1 + 15))
    def _phase2c():
        parts = spatial_parts(6)
        r = step - (P1 + 11)
        for gg in range(2):
            g8 = r * 2 + gg
            for c in range(NC):
                if parts and (gg * NC + c) in (0, 1, 3, 5, 6, 8):
                    parts.pop(0)()
                ls = slice(c * 128, (c + 1) * 128)
                X = [(zz_s[k1, pl.ds(pl.multiple_of(g8 * 16, 16), 8), ls],
                      zz_s[k1, pl.ds(pl.multiple_of(g8 * 16 + 8, 8), 8), ls]) for k1 in range(NK)]
                ys = _irfft_full(X)
                dd = ssmd_ref[:, ls].astype(F32)
                for n1 in range(NB):
                    rows = pl.ds(pl.multiple_of(n1 * N2 + g8 * 8, 8), 8)
                    s_s[rows, ls] = ys[n1] + x_s[0, rows, ls] * dd

    @pl.when(step == P1 + 15)
    def _phase2d():
        spatial()
        copies[2].wait()

    @pl.when(step >= P1 + P2)
    def _phase3():
        rows = pl.ds(pl.multiple_of((step - P1 - P2) * RB, RB), RB)
        o = _dot(z1_s[rows, :], wout_s[...])
        gate = o * jax.nn.sigmoid(o)
        o_ref[...] = (q_ref[...].astype(F32)
                      + xn_s[rows, :].astype(F32) * s_s[rows, :] * gate).astype(o_ref.dtype)


@jax.jit
def pallas_recurrent_scan__ssm_conv_h3__mixer_gmlp__prompt_kernel(
    A_q: jax.Array,
    A_k: jax.Array,
    A_v: jax.Array,
    A_shift_k: jax.Array,
    A_ssm_k: jax.Array,
    A_ssm_D: jax.Array,
    B_x: jax.Array,
    B_w_in: jax.Array,
    B_w_sp: jax.Array,
    B_b_sp: jax.Array,
    B_w_out: jax.Array,
):
    del B_x
    f = jnp.asarray(_F, BF16)
    g = jnp.asarray(_G, BF16)

    p1 = lambda i: jnp.minimum(i, P1 - 1)
    p2 = lambda i: jnp.clip(i - P1, 0, P2 - 1)
    p3 = lambda i: jnp.clip(i - P1 - P2, 0, P3 - 1)
    p13 = lambda i: jnp.where(i < P1 + P2, p1(i), p3(i))
    const = lambda shape: pl.BlockSpec(shape, lambda i: (0,) * len(shape))
    hbm = pl.BlockSpec(memory_space=pl.ANY)

    out = pl.pallas_call(
        _kernel,
        grid=(P1 + P2 + P3,),
        in_specs=[
            pl.BlockSpec((RB, D), lambda i: (p13(i), 0)),
            pl.BlockSpec((RB, D), lambda i: (p1(i), 0)),
            pl.BlockSpec((RB, D), lambda i: (p1(i), 0)),
            pl.BlockSpec((D, RB), lambda i: (0, p1(i))),
            const((4, D)),
            const((1, D)),
            const((D, 2 * FH)),
            pl.BlockSpec((RS, S), lambda i: (p2(i), 0)),
            pl.BlockSpec((None, 1, RS), lambda i: (p2(i), 0, 0)),
            hbm, hbm, hbm,
        ],
        out_specs=pl.BlockSpec((RB, D), lambda i: (p3(i), 0)),
        out_shape=jax.ShapeDtypeStruct((S, D), A_q.dtype),
        scratch_shapes=[
            pltpu.VMEM((S, FH), BF16),
            pltpu.VMEM((S, FH), BF16),
            pltpu.VMEM((S, D), BF16),
            pltpu.VMEM((2, S, D), F32),
            pltpu.VMEM((2, NK, 2 * N2, D), BF16),
            pltpu.VMEM((NK, 2 * N2, D), F32),
            pltpu.VMEM((S, D), F32),
            pltpu.VMEM((8, D), F32),
            pltpu.VMEM((NK, 2 * N2, 2 * N2), BF16),
            pltpu.VMEM((NK, 2 * N2, 2 * N2), BF16),
            pltpu.VMEM((FH, D), BF16),
            pltpu.SemaphoreType.DMA((3,)),
        ],
        compiler_params=pltpu.CompilerParams(
            dimension_semantics=("arbitrary",),
            vmem_limit_bytes=110 * 1024 * 1024,
        ),
    )(A_q.reshape(S, D), A_k.reshape(S, D), A_v.reshape(S, D), A_ssm_k, A_shift_k.T,
      A_ssm_D.reshape(1, D), B_w_in, B_w_sp, B_b_sp.reshape(P2, 1, RS), f, g, B_w_out)
    return out.reshape(A_q.shape)
```

```python
import functools
import math

import jax
import jax.numpy as jnp
import numpy as np
from jax import lax
import jax.experimental.pallas as pl
import jax.experimental.pallas.tpu as pltpu

S, D, FH = 2048, 640, 768
N1, N2 = 64, 64
NB = N1 // 2
NK = NB + 1
NC = D // 128
P1, P2, P3 = 8, 16, 8
RB = S // P1
RS = S // P2
F32, BF16 = jnp.float32, jnp.bfloat16


def _dft_mats():
    k1 = np.arange(NK)[:, None, None]
    k2 = np.arange(N2)[None, :, None]
    n2 = np.arange(N2)[None, None, :]
    m = np.exp(-2j * np.pi * (n2 * k1 / (N1 * N2) + n2 * k2 / N2))
    f = np.concatenate([np.concatenate([m.real, -m.imag], 2),
                        np.concatenate([m.imag, m.real], 2)], 1)
    perm = np.array([part * N2 + 8 * g + i for g in range(N2 // 8) for part in range(2) for i in range(8)])
    f = f[:, :, perm]
    g = np.transpose(f, (0, 2, 1)) / (N1 * N2)
    return f.astype(np.float32), g.astype(np.float32)


_F, _G = _dft_mats()


def _add(a, b):
    return b if a is None else a if b is None else a + b


def _sub(a, b):
    return (None if b is None else -b) if a is None else a if b is None else a - b


def _cmul(re, im, ang):
    c, s = float(np.float32(math.cos(ang))), float(np.float32(math.sin(ang)))
    if im is None:
        return re * c, re * s
    if abs(abs(c) - abs(s)) < 1e-6:
        if c * s > 0:
            return (re - im) * c, (re + im) * c
        return (re + im) * c, (im - re) * c
    return re * c - im * s, re * s + im * c


def _rfft(x, tick):
    n = len(x)
    if n == 16:
        tick()
    if n == 2:
        return [(_add(x[0], x[1]), None), (_sub(x[0], x[1]), None)]
    e, o = _rfft(x[0::2], tick), _rfft(x[1::2], tick)
    h = n // 2
    out = [None] * (h + 1)
    out[0] = (e[0][0] + o[0][0], None)
    out[h] = (e[0][0] - o[0][0], None)
    q = h // 2
    out[q] = (e[q][0], -o[q][0])
    for k in range(1, q):
        tr, ti = _cmul(o[k][0], o[k][1], -2 * math.pi * k / n)
        er, ei = e[k]
        out[k] = (er + tr, ei + ti)
        out[h - k] = (er - tr, ti - ei)
    return out


def _irfft_full(X, tick, need=None):
    n = 2 * (len(X) - 1)
    if n == 16:
        tick()
    need = n // 2 if need is None else need
    if n == 2:
        r = [X[0][0] + X[1][0]]
        if need > 1:
            r.append(X[0][0] - X[1][0])
        return r
    h, q = n // 2, n // 4
    e, o = [None] * (q + 1), [None] * (q + 1)
    e[0] = (X[0][0] + X[h][0], None)
    o[0] = (X[0][0] - X[h][0], None)
    e[q] = (X[q][0] * 2.0, None)
    o[q] = (X[q][1] * -2.0, None)
    for k in range(1, q):
        (ar, ai), (br, bi) = X[k], X[h - k]
        e[k] = (ar + br, ai - bi)
        o[k] = _cmul(ar - br, ai + bi, 2 * math.pi * k / n)
    xe, xo = _irfft_full(e, tick, need // 2), _irfft_full(o, tick, need // 2)
    out = [None] * need
    out[0::2], out[1::2] = xe, xo
    return out


def _ln(x):
    m = jnp.mean(x, axis=-1, keepdims=True)
    c = x - m
    v = jnp.mean(c * c, axis=-1, keepdims=True)
    return c * lax.rsqrt(v + 1e-5)


def _gelu(x):
    return 0.5 * x * (1.0 + jnp.tanh(0.7978845608028654 * (x + 0.044715 * x * x * x)))


def _dot(a, b):
    return jnp.dot(a, b, preferred_element_type=F32)


def _kernel(q_ref, k_ref, v_ref, sk_ref, shift_ref, ssmd_ref, win_ref, wsp_ref, bsp_ref,
            f_hbm, g_hbm, wout_hbm,
            o_ref,
            z1_s, z2_s, xn_s, x_s, a_s, zz_s, s_s, tail_s, f_s, g_s, wout_s, sem):
    step = pl.program_id(0)
    copies = [pltpu.make_async_copy(f_hbm, f_s, sem.at[0]),
              pltpu.make_async_copy(g_hbm, g_s, sem.at[1]),
              pltpu.make_async_copy(wout_hbm, wout_s, sem.at[2])]

    @pl.when(step == 0)
    def _start():
        tail_s[...] = jnp.zeros_like(tail_s)

    @pl.when(step == 1)
    def _start2():
        for cp in copies:
            cp.start()

    @pl.when(step < P1)
    def _phase1():
        row0 = pl.multiple_of(step * RB, RB)
        rows = pl.ds(row0, RB)
        w = shift_ref[...].astype(F32)

        for h in range(2):
            hs = slice(h * 128, (h + 1) * 128)
            hr = pl.ds(pl.multiple_of(step * RB + h * 128, 128), 128)
            xn = _ln(q_ref[hs, :].astype(F32)).astype(BF16)
            xn_s[hr, :] = xn

            def kv(c):
                ls = slice(c * 128, (c + 1) * 128)
                kf = k_ref[hs, ls].astype(F32)
                ext = jnp.concatenate([tail_s[:, ls], kf], 0)
                ks = kf * w[0:1, ls]
                for j in range(1, 4):
                    ks = ks + ext[8 - j:8 - j + 128] * w[j:j + 1, ls]
                tail_s[:, ls] = kf[120:]
                x_s[0, hr, ls] = ks * v_ref[hs, ls].astype(F32)
                x_s[1, hr, ls] = sk_ref[ls, hs].astype(F32).T

            z2 = []
            for j in range(12):
                cs = slice(j * 128, (j + 1) * 128)
                z = _gelu(_dot(xn, win_ref[:, cs]))
                if j < 6:
                    z1_s[hr, cs] = z.astype(BF16)
                else:
                    z2.append(z)
                if j % 2 == 0 and j < 10:
                    kv(j // 2)
            z2_s[hr, :] = _ln(jnp.concatenate(z2, 1)).astype(BF16)

    def spatial_parts(n):
        r = step - P1
        rows = pl.ds(pl.multiple_of(r * RS, RS), RS)
        bcol = jnp.broadcast_to(bsp_ref[...].astype(F32), (RS, RS)).T
        wd = FH // n

        def part(j):
            cs = slice(j * wd, (j + 1) * wd)
            gate = _dot(wsp_ref[...], z2_s[:, cs]) + jnp.concatenate([bcol] * (wd // RS), 1)
            z1_s[rows, cs] = (z1_s[rows, cs].astype(F32) * gate).astype(BF16)
        return [functools.partial(part, j) for j in range(n)]

    def spatial_gen():
        r = step - P1
        rows = pl.ds(pl.multiple_of(r * RS, RS), RS)
        bcol = jnp.broadcast_to(bsp_ref[...].astype(F32), (RS, RS)).T
        for j in range(FH // 128):
            cs = slice(j * 128, (j + 1) * 128)
            acc = bcol
            for kk in range(4):
                ks_ = slice(kk * 512, (kk + 1) * 512)
                acc = acc + _dot(wsp_ref[:, ks_], z2_s[ks_, cs])
                if kk == 3:
                    z1_s[rows, cs] = (z1_s[rows, cs].astype(F32) * acc).astype(BF16)
                yield

    def ticker(nticks):
        gen = spatial_gen()
        state = {"t": 0, "done": 0}

        def tick():
            state["t"] += 1
            while state["done"] < 24 and state["done"] * nticks < state["t"] * 24:
                next(gen)
                state["done"] += 1
        return tick

    def spatial():
        spatial_parts(1)[0]()

    @pl.when(jnp.logical_and(step >= P1, step < P1 + 8))
    def _phase2a():
        tick = ticker(40)
        r = step - P1
        which = r // 4
        for gg in range(2):
            g8 = (r % 4) * 2 + gg
            for c in range(NC):
                ls = slice(c * 128, (c + 1) * 128)
                xs = [x_s[which, pl.ds(pl.multiple_of(n1 * N2 + g8 * 8, 8), 8), ls] for n1 in range(NB)]
                X = _rfft(xs + [None] * NB, tick)
                for k1 in range(NK):
                    re, im = X[k1]
                    im = jnp.zeros_like(re) if im is None else im
                    a_s[which, k1, pl.ds(pl.multiple_of(g8 * 16, 16), 16), ls] = (
                        jnp.concatenate([re, im], 0).astype(BF16))

    @pl.when(step == P1 + 8)
    def _wait_fg():
        copies[0].wait()
        copies[1].wait()

    @pl.when(jnp.logical_and(step >= P1 + 8, step < P1 + 11))
    def _phase2b():
        tick = ticker(11)
        r = step - (P1 + 8)
        for u in range(11):
            k1 = r * 11 + u
            f = f_s[k1]
            xk = _dot(f, a_s[0, k1])
            xf = _dot(f, a_s[1, k1])
            tick()
            kr, ki, fr, fi = xk[:N2], xk[N2:], xf[:N2], xf[N2:]
            y = jnp.concatenate([kr * fr - ki * fi, kr * fi + ki * fr], 0).astype(BF16)
            zz_s[k1] = _dot(g_s[k1], y)

    @pl.when(jnp.logical_and(step >= P1 + 11, step < P1 + 15))
    def _phase2c():
        tick = ticker(40)
        r = step - (P1 + 11)
        for gg in range(2):
            g8 = r * 2 + gg
            for c in range(NC):
                ls = slice(c * 128, (c + 1) * 128)
                X = [(zz_s[k1, pl.ds(pl.multiple_of(g8 * 16, 16), 8), ls],
                      zz_s[k1, pl.ds(pl.multiple_of(g8 * 16 + 8, 8), 8), ls]) for k1 in range(NK)]
                ys = _irfft_full(X, tick)
                dd = ssmd_ref[:, ls].astype(F32)
                for n1 in range(NB):
                    rows = pl.ds(pl.multiple_of(n1 * N2 + g8 * 8, 8), 8)
                    s_s[rows, ls] = ys[n1] + x_s[0, rows, ls] * dd

    @pl.when(step == P1 + 15)
    def _phase2d():
        spatial()
        copies[2].wait()

    @pl.when(step >= P1 + P2)
    def _phase3():
        rows = pl.ds(pl.multiple_of((step - P1 - P2) * RB, RB), RB)
        o = _dot(z1_s[rows, :], wout_s[...])
        gate = o * jax.nn.sigmoid(o)
        o_ref[...] = (q_ref[...].astype(F32)
                      + xn_s[rows, :].astype(F32) * s_s[rows, :] * gate).astype(o_ref.dtype)


@jax.jit
def pallas_recurrent_scan__ssm_conv_h3__mixer_gmlp__prompt_kernel(
    A_q: jax.Array,
    A_k: jax.Array,
    A_v: jax.Array,
    A_shift_k: jax.Array,
    A_ssm_k: jax.Array,
    A_ssm_D: jax.Array,
    B_x: jax.Array,
    B_w_in: jax.Array,
    B_w_sp: jax.Array,
    B_b_sp: jax.Array,
    B_w_out: jax.Array,
):
    del B_x
    f = jnp.asarray(_F, BF16)
    g = jnp.asarray(_G, BF16)

    p1 = lambda i: jnp.minimum(i, P1 - 1)
    p2 = lambda i: jnp.clip(i - P1, 0, P2 - 1)
    p3 = lambda i: jnp.clip(i - P1 - P2, 0, P3 - 1)
    p13 = lambda i: jnp.where(i < P1 + P2, p1(i), p3(i))
    const = lambda shape: pl.BlockSpec(shape, lambda i: (0,) * len(shape))
    hbm = pl.BlockSpec(memory_space=pl.ANY)

    out = pl.pallas_call(
        _kernel,
        grid=(P1 + P2 + P3,),
        in_specs=[
            pl.BlockSpec((RB, D), lambda i: (p13(i), 0)),
            pl.BlockSpec((RB, D), lambda i: (p1(i), 0)),
            pl.BlockSpec((RB, D), lambda i: (p1(i), 0)),
            pl.BlockSpec((D, RB), lambda i: (0, p1(i))),
            const((4, D)),
            const((1, D)),
            const((D, 2 * FH)),
            pl.BlockSpec((RS, S), lambda i: (p2(i), 0)),
            pl.BlockSpec((None, 1, RS), lambda i: (p2(i), 0, 0)),
            hbm, hbm, hbm,
        ],
        out_specs=pl.BlockSpec((RB, D), lambda i: (p3(i), 0)),
        out_shape=jax.ShapeDtypeStruct((S, D), A_q.dtype),
        scratch_shapes=[
            pltpu.VMEM((S, FH), BF16),
            pltpu.VMEM((S, FH), BF16),
            pltpu.VMEM((S, D), BF16),
            pltpu.VMEM((2, S, D), F32),
            pltpu.VMEM((2, NK, 2 * N2, D), BF16),
            pltpu.VMEM((NK, 2 * N2, D), F32),
            pltpu.VMEM((S, D), F32),
            pltpu.VMEM((8, D), F32),
            pltpu.VMEM((NK, 2 * N2, 2 * N2), BF16),
            pltpu.VMEM((NK, 2 * N2, 2 * N2), BF16),
            pltpu.VMEM((FH, D), BF16),
            pltpu.SemaphoreType.DMA((3,)),
        ],
        compiler_params=pltpu.CompilerParams(
            dimension_semantics=("arbitrary",),
            vmem_limit_bytes=110 * 1024 * 1024,
        ),
    )(A_q.reshape(S, D), A_k.reshape(S, D), A_v.reshape(S, D), A_ssm_k, A_shift_k.T,
      A_ssm_D.reshape(1, D), B_w_in, B_w_sp, B_b_sp.reshape(P2, 1, RS), f, g, B_w_out)
    return out.reshape(A_q.shape)
```

```python
import functools
import math

import jax
import jax.numpy as jnp
import numpy as np
from jax import lax
import jax.experimental.pallas as pl
import jax.experimental.pallas.tpu as pltpu

S, D, FH = 2048, 640, 768
N1, N2 = 64, 64
NB = N1 // 2
NK = NB + 1
NC = D // 128
P1, P2, P3 = 8, 16, 8
RB = S // P1
RS = S // P2
F32, BF16 = jnp.float32, jnp.bfloat16


def _dft_mats():
    k1 = np.arange(NK)[:, None, None]
    k2 = np.arange(N2)[None, :, None]
    n2 = np.arange(N2)[None, None, :]
    m = np.exp(-2j * np.pi * (n2 * k1 / (N1 * N2) + n2 * k2 / N2))
    f = np.concatenate([np.concatenate([m.real, -m.imag], 2),
                        np.concatenate([m.imag, m.real], 2)], 1)
    perm = np.array([part * N2 + 8 * g + i for g in range(N2 // 8) for part in range(2) for i in range(8)])
    f = f[:, :, perm]
    g = np.transpose(f, (0, 2, 1)) / (N1 * N2)
    return f.astype(np.float32), g.astype(np.float32)


_F, _G = _dft_mats()


def _add(a, b):
    return b if a is None else a if b is None else a + b


def _sub(a, b):
    return (None if b is None else -b) if a is None else a if b is None else a - b


def _cmul(re, im, ang):
    c, s = float(np.float32(math.cos(ang))), float(np.float32(math.sin(ang)))
    if im is None:
        return re * c, re * s
    if abs(abs(c) - abs(s)) < 1e-6:
        if c * s > 0:
            return (re - im) * c, (re + im) * c
        return (re + im) * c, (im - re) * c
    return re * c - im * s, re * s + im * c


def _rfft(x, tick):
    n = len(x)
    if n == 16:
        tick()
    if n == 2:
        return [(_add(x[0], x[1]), None), (_sub(x[0], x[1]), None)]
    e, o = _rfft(x[0::2], tick), _rfft(x[1::2], tick)
    h = n // 2
    out = [None] * (h + 1)
    out[0] = (e[0][0] + o[0][0], None)
    out[h] = (e[0][0] - o[0][0], None)
    q = h // 2
    out[q] = (e[q][0], -o[q][0])
    for k in range(1, q):
        tr, ti = _cmul(o[k][0], o[k][1], -2 * math.pi * k / n)
        er, ei = e[k]
        out[k] = (er + tr, ei + ti)
        out[h - k] = (er - tr, ti - ei)
    return out


def _irfft_full(X, tick, need=None):
    n = 2 * (len(X) - 1)
    if n == 16:
        tick()
    need = n // 2 if need is None else need
    if n == 2:
        r = [X[0][0] + X[1][0]]
        if need > 1:
            r.append(X[0][0] - X[1][0])
        return r
    h, q = n // 2, n // 4
    e, o = [None] * (q + 1), [None] * (q + 1)
    e[0] = (X[0][0] + X[h][0], None)
    o[0] = (X[0][0] - X[h][0], None)
    e[q] = (X[q][0] * 2.0, None)
    o[q] = (X[q][1] * -2.0, None)
    for k in range(1, q):
        (ar, ai), (br, bi) = X[k], X[h - k]
        e[k] = (ar + br, ai - bi)
        o[k] = _cmul(ar - br, ai + bi, 2 * math.pi * k / n)
    xe, xo = _irfft_full(e, tick, need // 2), _irfft_full(o, tick, need // 2)
    out = [None] * need
    out[0::2], out[1::2] = xe, xo
    return out


def _ln(x):
    m = jnp.mean(x, axis=-1, keepdims=True)
    c = x - m
    v = jnp.mean(c * c, axis=-1, keepdims=True)
    return c * lax.rsqrt(v + 1e-5)


def _gelu(x):
    return 0.5 * x * (1.0 + jnp.tanh(0.7978845608028654 * (x + 0.044715 * x * x * x)))


def _dot(a, b):
    return jnp.dot(a, b, preferred_element_type=F32)


def _kernel(q_hbm, k_hbm, v_hbm, sk_hbm, shift_ref, ssmd_ref, win_hbm, wsp_hbm, bsp_ref,
            f_hbm, g_hbm, wout_hbm,
            o_hbm,
            q_s, k_s, v_s, sk_s, win_s, wsp_s, o_s,
            z1_s, z2_s, xn_s, x_s, a_s, zz_s, s_s, tail_s, f_s, g_s, wout_s, sem):
    def blk(i, n):
        return pl.ds(i * n if isinstance(i, int) else pl.multiple_of(i * n, n), n)

    def in_copy(t, i):
        if t == 3:
            return pltpu.make_async_copy(sk_hbm.at[:, blk(i, RB)], sk_s.at[i], sem.at[3 * P1 + i])
        src, dst = ((q_hbm, q_s), (k_hbm, k_s), (v_hbm, v_s))[t]
        return pltpu.make_async_copy(src.at[blk(i, RB)], dst.at[blk(i, RB)], sem.at[t * P1 + i])

    def wsp_copy(i):
        return pltpu.make_async_copy(wsp_hbm.at[blk(i, RS)], wsp_s.at[i], sem.at[4 * P1 + i])

    def out_copy(i):
        return pltpu.make_async_copy(o_s.at[blk(i, RB)], o_hbm.at[blk(i, RB)], sem.at[4 * P1 + P2 + i])

    base = 4 * P1 + P2 + P3
    win_copy, f_copy, g_copy, wout_copy = [
        pltpu.make_async_copy(a, b, sem.at[base + i])
        for i, (a, b) in enumerate(((win_hbm, win_s), (f_hbm, f_s), (g_hbm, g_s), (wout_hbm, wout_s)))]

    gstep = pl.program_id(0)

    def loop(lo, n):
        def deco(f):
            @pl.when(jnp.logical_and(gstep >= lo, gstep < lo + n))
            def _():
                f(gstep - lo)
        return deco

    @pl.when(gstep == 0)
    def _():
      in_copy(0, 0).start()
      win_copy.start()
      for i in range(P1):
          for t in range(4):
              if (t, i) != (0, 0):
                  in_copy(t, i).start()
      f_copy.start()
      g_copy.start()
      wout_copy.start()
      tail_s[...] = jnp.zeros_like(tail_s)
      win_copy.wait()

    @loop(0, P1)
    def _phase1(step):
        for t in range(4):
            in_copy(t, step).wait()
        q_ref, k_ref, v_ref = (a.at[blk(step, RB)] for a in (q_s, k_s, v_s))
        sk_ref, win_ref = sk_s.at[step], win_s
        w = shift_ref[...].astype(F32)

        for h in range(2):
            hs = slice(h * 128, (h + 1) * 128)
            hr = pl.ds(pl.multiple_of(step * RB + h * 128, 128), 128)
            xn = _ln(q_ref[hs, :].astype(F32)).astype(BF16)
            xn_s[hr, :] = xn

            def kv(c):
                ls = slice(c * 128, (c + 1) * 128)
                kf = k_ref[hs, ls].astype(F32)
                ext = jnp.concatenate([tail_s[:, ls], kf], 0)
                ks = kf * w[0:1, ls]
                for j in range(1, 4):
                    ks = ks + ext[8 - j:8 - j + 128] * w[j:j + 1, ls]
                tail_s[:, ls] = kf[120:]
                x_s[0, hr, ls] = ks * v_ref[hs, ls].astype(F32)
                x_s[1, hr, ls] = sk_ref[ls, hs].astype(F32).T

            z2 = []
            for j in range(12):
                cs = slice(j * 128, (j + 1) * 128)
                z = _gelu(_dot(xn, win_ref[:, cs]))
                if j < 6:
                    z1_s[hr, cs] = z.astype(BF16)
                else:
                    z2.append(z)
                if j % 2 == 0 and j < 10:
                    kv(j // 2)
            z2_s[hr, :] = _ln(jnp.concatenate(z2, 1)).astype(BF16)

    def spatial_gen(r):
        wsp_ref = wsp_hbm
        rows = pl.ds(pl.multiple_of(r * RS, RS), RS)
        bcol = jnp.broadcast_to(bsp_ref[r].astype(F32), (RS, RS)).T
        for j in range(FH // 128):
            cs = slice(j * 128, (j + 1) * 128)
            acc = bcol
            for kk in range(4):
                ks_ = slice(kk * 512, (kk + 1) * 512)
                acc = acc + _dot(wsp_ref[:, ks_], z2_s[ks_, cs])
                if kk == 3:
                    z1_s[rows, cs] = (z1_s[rows, cs].astype(F32) * acc).astype(BF16)
                yield

    def ticker(r, nticks):
        gen = spatial_gen(r)
        state = {"t": 0, "done": 0}

        def tick():
            state["t"] += 1
            while state["done"] < 24 and state["done"] * nticks < state["t"] * 24:
                next(gen)
                state["done"] += 1
        return tick

    @loop(8, 8)
    def _phase2a(r):
        tick = ticker(r, 40)
        which = r // 4
        for gg in range(2):
            g8 = (r % 4) * 2 + gg
            for c in range(NC):
                ls = slice(c * 128, (c + 1) * 128)
                xs = [x_s[which, pl.ds(pl.multiple_of(n1 * N2 + g8 * 8, 8), 8), ls] for n1 in range(NB)]
                X = _rfft(xs + [None] * NB, tick)
                for k1 in range(NK):
                    re, im = X[k1]
                    im = jnp.zeros_like(re) if im is None else im
                    a_s[which, k1, pl.ds(pl.multiple_of(g8 * 16, 16), 16), ls] = (
                        jnp.concatenate([re, im], 0).astype(BF16))

    @pl.when(gstep == 16)
    def _():
        f_copy.wait()
        g_copy.wait()

    @loop(16, 3)
    def _phase2b(r):
        tick = ticker(r + 8, 11)
        for u in range(11):
            k1 = r * 11 + u
            f = f_s[k1]
            xk = _dot(f, a_s[0, k1])
            xf = _dot(f, a_s[1, k1])
            tick()
            kr, ki, fr, fi = xk[:N2], xk[N2:], xf[:N2], xf[N2:]
            y = jnp.concatenate([kr * fr - ki * fi, kr * fi + ki * fr], 0).astype(BF16)
            zz_s[k1] = _dot(g_s[k1], y)

    @loop(19, 4)
    def _phase2c(r):
        tick = ticker(r + 11, 40)
        for gg in range(2):
            g8 = r * 2 + gg
            for c in range(NC):
                ls = slice(c * 128, (c + 1) * 128)
                X = [(zz_s[k1, pl.ds(pl.multiple_of(g8 * 16, 16), 8), ls],
                      zz_s[k1, pl.ds(pl.multiple_of(g8 * 16 + 8, 8), 8), ls]) for k1 in range(NK)]
                ys = _irfft_full(X, tick)
                dd = ssmd_ref[:, ls].astype(F32)
                for n1 in range(NB):
                    rows = pl.ds(pl.multiple_of(n1 * N2 + g8 * 8, 8), 8)
                    s_s[rows, ls] = ys[n1] + x_s[0, rows, ls] * dd

    @pl.when(gstep == 23)
    def _():
        ticker(15, 1)()
        wout_copy.wait()

    @loop(24, P3)
    def _phase3(i):
        rows = blk(i, RB)
        o = _dot(z1_s[rows, :], wout_s[...])
        gate = o * jax.nn.sigmoid(o)
        o_s[rows, :] = (q_s[rows, :].astype(F32)
                        + xn_s[rows, :].astype(F32) * s_s[rows, :] * gate).astype(o_s.dtype)
        out_copy(i).start()

    @pl.when(gstep == 31)
    def _():
        for i in range(P3):
            out_copy(i).wait()


@jax.jit
def pallas_recurrent_scan__ssm_conv_h3__mixer_gmlp__prompt_kernel(
    A_q: jax.Array,
    A_k: jax.Array,
    A_v: jax.Array,
    A_shift_k: jax.Array,
    A_ssm_k: jax.Array,
    A_ssm_D: jax.Array,
    B_x: jax.Array,
    B_w_in: jax.Array,
    B_w_sp: jax.Array,
    B_b_sp: jax.Array,
    B_w_out: jax.Array,
):
    del B_x
    f = jnp.asarray(_F, BF16)
    g = jnp.asarray(_G, BF16)

    hbm = pl.BlockSpec(memory_space=pl.ANY)
    vmem = pl.BlockSpec(memory_space=pltpu.VMEM)

    out = pl.pallas_call(
        _kernel,
        grid=(32,),
        in_specs=[hbm, hbm, hbm, hbm, vmem, vmem, hbm,
                  pl.BlockSpec((RS, S), lambda i: (jnp.clip(i - P1, 0, P2 - 1), 0)), vmem, hbm, hbm, hbm],
        out_specs=hbm,
        out_shape=jax.ShapeDtypeStruct((S, D), A_q.dtype),
        scratch_shapes=[
            pltpu.VMEM((S, D), BF16),
            pltpu.VMEM((S, D), BF16),
            pltpu.VMEM((S, D), BF16),
            pltpu.VMEM((P1, D, RB), BF16),
            pltpu.VMEM((D, 2 * FH), BF16),
            pltpu.VMEM((8, 128), BF16),
            pltpu.VMEM((S, D), BF16),
            pltpu.VMEM((S, FH), BF16),
            pltpu.VMEM((S, FH), BF16),
            pltpu.VMEM((S, D), BF16),
            pltpu.VMEM((2, S, D), F32),
            pltpu.VMEM((2, NK, 2 * N2, D), BF16),
            pltpu.VMEM((NK, 2 * N2, D), F32),
            pltpu.VMEM((S, D), F32),
            pltpu.VMEM((8, D), F32),
            pltpu.VMEM((NK, 2 * N2, 2 * N2), BF16),
            pltpu.VMEM((NK, 2 * N2, 2 * N2), BF16),
            pltpu.VMEM((FH, D), BF16),
            pltpu.SemaphoreType.DMA((4 * P1 + P2 + P3 + 4,)),
        ],
        compiler_params=pltpu.CompilerParams(
            vmem_limit_bytes=110 * 1024 * 1024,
        ),
    )(A_q.reshape(S, D), A_k.reshape(S, D), A_v.reshape(S, D), A_ssm_k, A_shift_k.T,
      A_ssm_D.reshape(1, D), B_w_in, B_w_sp, B_b_sp.reshape(P2, 1, RS), f, g, B_w_out)
    return out.reshape(A_q.shape)
```
